```python
import jax
import jax.numpy as jnp

def _softmax(x, axis=-1):
    return jax.nn.softmax(x, axis=axis)
def _gelu(x):
    return jax.nn.gelu(x, approximate=True)
def _silu(x):
    return jax.nn.silu(x)
def _sigmoid(x):
    return jax.nn.sigmoid(x)
def _layernorm(x, axis=-1, eps=1e-5):
    m = jnp.mean(x, axis=axis, keepdims=True)
    v = jnp.var(x, axis=axis, keepdims=True)
    return (x - m) / jnp.sqrt(v + eps)
def _scatter_add(tgt, idx, src, axis=0):
    return tgt.at[idx].add(src)
def _segment_sum(src, seg, n):
    return jax.ops.segment_sum(src, seg, n)
class _Rng:
    def __init__(self, key):
        self._k = key
    def _next(self):
        self._k, sub = jax.random.split(self._k)
        return sub
    def normal(self, shape):
        return jax.random.normal(self._next(), shape, dtype=jnp.bfloat16)
    def randint(self, lo, hi, shape):
        return jax.random.randint(self._next(), shape, lo, hi, dtype=jnp.int32)
    def uniform(self, shape, lo=0.0, hi=1.0):
        return jax.random.uniform(self._next(), shape, jnp.bfloat16, lo, hi)
    def permutation(self, n):
        return jax.random.permutation(self._next(), n)


kernel_name = 'concat_heads__sliding_block_cached__compressed_kv_cla__decode'

def setup_inputs():
    _rng = _Rng(jax.random.key(int.from_bytes(__import__("os").urandom(4), "little")))
    _w = (lambda a: (lambda t: t.astype(jnp.bfloat16) if jnp.issubdtype(t.dtype, jnp.floating) else t)(jnp.asarray(a)))
    def _A_setup():
        B, Sq, D = 4, 1, 512
        Hq, Hkv, Sk, Dh = 32, 32, 4096, 128
        assert Hq % Hkv == 0, (Hq, Hkv)
        return {
            "x": _w((lambda *s: _rng.normal(s) * 0.05)(B, Sq, D)),
            "k_cache": _w((lambda *s: _rng.normal(s) * 0.05)(B, Hkv, Sk, Dh)),
            "v_cache": _w((lambda *s: _rng.normal(s) * 0.05)(B, Hkv, Sk, Dh)),
            "wq": _w((lambda *s: _rng.normal(s) * 0.05)(D, Hq * Dh) * (D ** -0.5)),
            "wo": _w((lambda *s: _rng.normal(s) * 0.05)(Hq * Dh, D) * ((Hq * Dh) ** -0.5)),
        }
    _A_in = _A_setup()

    def _B_setup():
        B, H, Sq, Sk, D, M = 4, 32, 1, 4096, 128, 512
        Dc = 4 * D
        return {
            "x": _w((lambda *s: _rng.normal(s) * 0.05)(B, Sq, M)),
            "c_kv": _w((lambda *s: _rng.normal(s) * 0.05)(B, Sk, Dc)),
            "w_q": _w((lambda *s: _rng.normal(s) * 0.05)(M, H, D) * (M ** -0.5)),
            "w_uk": _w((lambda *s: _rng.normal(s) * 0.05)(Dc, H, D) * (Dc ** -0.5)),
            "w_uv": _w((lambda *s: _rng.normal(s) * 0.05)(Dc, H, D) * (Dc ** -0.5)),
            "w_o": _w((lambda *s: _rng.normal(s) * 0.05)(H, D, M) * ((H * D) ** -0.5)),
        }
    _B_in = _B_setup()

    return {
        "A_x": _A_in["x"],
        "A_k_cache": _A_in["k_cache"],
        "A_v_cache": _A_in["v_cache"],
        "A_wq": _A_in["wq"],
        "A_wo": _A_in["wo"],
        "B_x": _B_in["x"],
        "B_c_kv": _B_in["c_kv"],
        "B_w_q": _B_in["w_q"],
        "B_w_uk": _B_in["w_uk"],
        "B_w_uv": _B_in["w_uv"],
        "B_w_o": _B_in["w_o"],
    }

def reference(A_x, A_k_cache, A_v_cache, A_wq, A_wo, B_x, B_c_kv, B_w_q, B_w_uk, B_w_uv, B_w_o):
    def _A_ref(x, k_cache, v_cache, wq, wo):
        B, Sq, D = x.shape
        Hq, Dh = 32, 128
        Hkv, Sk = k_cache.shape[1], k_cache.shape[2]
        W = min(4096, max(256, Sk // 4))
        rep = Hq // Hkv
        q = (lambda x, *d: x.transpose(*d))((x @ wq).reshape(B, Sq, Hq, Dh), 0, 2, 1, 3)
        k = jnp.repeat(k_cache[:, :, Sk - W:, :], rep, axis=1)
        v = jnp.repeat(v_cache[:, :, Sk - W:, :], rep, axis=1)
        scores = jnp.einsum("bhqd,bhkd->bhqk", q, k) * (Dh ** -0.5)
        p = _softmax(scores, axis=-1)
        o = jnp.einsum("bhqk,bhkd->bhqd", p, v)
        return (lambda x, *d: x.transpose(*d))(o, 0, 2, 1, 3).reshape(B, Sq, Hq * Dh) @ wo

    def _B_ref(x, c_kv, w_q, w_uk, w_uv, w_o):
        B, Sq, M = x.shape[0], x.shape[1], x.shape[2]
        Sk = c_kv.shape[1]
        H, D = w_q.shape[1], w_q.shape[2]
        q = jnp.einsum("bqm,mhd->bhqd", x, w_q)
        k = jnp.einsum("bkc,chd->bhkd", c_kv, w_uk)
        v = jnp.einsum("bkc,chd->bhkd", c_kv, w_uv)
        scores = jnp.einsum("bhqd,bhkd->bhqk", q, k) * (D ** -0.5)
        off = Sk - Sq
        qi = jnp.arange(Sq)[:, None]
        kj = jnp.arange(Sk)[None, :]
        cmask = kj <= (qi + off)
        scores = jnp.where(cmask[None, None], scores, -1e9)
        p = _softmax(scores, axis=-1)
        ctx = jnp.einsum("bhqk,bhkd->bhqd", p, v)
        return jnp.einsum("bhqd,hdm->bqm", ctx, w_o)

    a = _A_ref(A_x, A_k_cache, A_v_cache, A_wq, A_wo)
    b = _B_ref(B_x, B_c_kv, B_w_q, B_w_uk, B_w_uv, B_w_o)
    return jnp.concatenate([a, b], axis=-1)
```

```python
import functools

import jax
import jax.numpy as jnp
from jax import lax
import jax.experimental.pallas as pl
import jax.experimental.pallas.tpu as pltpu

B, H, DH, DM, SK, WIN, DC = 4, 32, 128, 512, 4096, 1024, 512
BF, F32 = jnp.bfloat16, jnp.float32
NT = (((1,), (1,)), ((), ()))
SCALE = DH ** -0.5

PIECE = 16 * 1024
NQ = 16
S_W1, S_W2, S_C, S_KV, S_WO, S_END = 0, 16, 32, 64, 192, 208


def _dot(a, b):
    return jnp.dot(a, b, preferred_element_type=F32)


def _dot_nt(a, b):
    return lax.dot_general(a, b, NT, preferred_element_type=F32)


def make_kernel(do_dma=True, do_compute=True, pr="0011", wways=4, cways=8, hways=8, lead=4, last_issue=4):
    prs = [int(pr[i % len(pr)]) for i in range(2 * NQ)]

    def kernel(ax_h, k_h, v_h, wq_h, wo_h, bx_h, c_h, bwq_h, wuk_h, wuv_h, bwo_h, out_ref,
               kb, vb, cb, wqb, wob, bwqb, wukb, wuvb, bwob, xb,
               qa_s, qabs_s, cc_s, ctx_s, o_s, s_s,
               sem_x, sem_w, sem_c, sem_kv, sem_o):

        def burst(desc):
            if not do_dma:
                return
            cnt = [0, 0]
            for p in prs:
                src, dst, sem = desc(p, cnt[p])
                cnt[p] += 1
                pltpu.make_async_copy(src, dst, sem).start(priority=p)

        def spread(t, i, n, ways):
            return (i % ways) * (n // ways) + t * (NQ // ways) + i // ways

        def rows128(src, dst, sem, t, i):
            r = pl.ds(pl.multiple_of(spread(t, i, 256, wways) * 32, 32), 32)
            return src.bitcast(jnp.uint32).at[r], dst.at[r], sem

        def issue_w1(t):
            burst(lambda p, i: rows128((bwq_h, wuk_h)[p], (bwqb, wukb)[p], sem_w.at[p], t, i))

        def issue_w2(t):
            def desc(p, i):
                if p == 1:
                    return rows128(wuv_h, wuvb, sem_w.at[3], t, i)
                w = i % wways
                n = i // wways
                per = NQ // wways
                if per >= 8:
                    rt = w * (32 // wways) + t * (per // 8) + n // 8
                    ct = n % 8
                else:
                    rt = w * (32 // wways) + lax.div(t, 8 // per)
                    ct = lax.rem(t, 8 // per) * per + n
                r = pl.ds(pl.multiple_of(rt * 16, 16), 16)
                cc = pl.ds(pl.multiple_of(ct * 512, 512), 512)
                return wq_h.at[r, cc], wqb.at[r, cc], sem_w.at[2]
            burst(desc)

        def issue_c(t):
            b = lax.shift_right_logical(t, 3)
            j = t & 7

            def desc(p, i):
                ways = cways
                g = p * ways + i % ways
                per = NQ // ways
                src = b * SK + g * (SK // (2 * ways)) + (j * per + i // ways) * 16
                dst = t * 512 + (p * NQ + i) * 16
                return (c_h.at[pl.ds(pl.multiple_of(src, 16), 16)],
                        cb.at[pl.ds(pl.multiple_of(dst, 16), 16)], sem_c.at[t & 7])
            burst(desc)

        def issue_kv(t):
            g = lax.shift_right_logical(t, 3)
            j = t & 7

            def desc(p, i):
                if hways == 8:
                    h = g * 8 + i % 8
                    r = (j * 2 + i // 8) * 64
                elif hways == 4:
                    h = g * 8 + (j & 4) + i % 4
                    r = ((j & 3) * 4 + i // 4) * 64
                r = pl.multiple_of(r, 64)
                return ((k_h, v_h)[p].at[h, pl.ds(SK - WIN + r, 64)],
                        (kb, vb)[p].at[h, pl.ds(r, 64)], sem_kv.at[p, g & 1])
            burst(desc)

        def issue_wo(t):
            def desc(p, i):
                r = pl.ds(pl.multiple_of(t * 128 + (i % 2) * 2048 + (i // 2) * 16, 16), 16)
                d = pl.ds(pl.multiple_of(t * 256 + (i % 2) * 128 + (i // 2) * 16, 16), 16)
                return (wo_h, bwo_h)[p].at[r], (wob, bwob)[p].at[d], sem_o.at[p, t]
            burst(desc)

        phases = [(S_W1, S_W2, issue_w1), (S_W2, S_C, issue_w2), (S_C, S_KV, issue_c),
                  (S_KV, S_WO, issue_kv), (S_WO, S_END, issue_wo)]

        def issue(s, lo, hi):
            for a, e, f in phases:
                if e <= lo or a >= hi:
                    continue
                if a <= lo and hi <= e:
                    f(s - a)
                elif a <= lo:
                    pl.when(s < e)(functools.partial(f, s - a))
                elif hi <= e:
                    pl.when(s >= a)(functools.partial(f, s - a))
                else:
                    pl.when(jnp.logical_and(s >= a, s < e))(functools.partial(f, s - a))

        def wait(ref, sem):
            if do_dma:
                pltpu.make_async_copy(ref, ref, sem).wait()

        def head_pair(w_ref, i):
            w = w_ref[pl.ds(i, 512, stride=16), :]
            lo = pltpu.bitcast(w << 16, F32).astype(BF)
            hi = pltpu.bitcast(w & jnp.uint32(0xFFFF0000), F32).astype(BF)
            return lo, hi

        def pro(s, c):
            issue(s, 0, S_W2 + lead)
            return c
        lax.fori_loop(0, 1, pro, 0)
        xa_cp = pltpu.make_async_copy(ax_h, xb.at[0], sem_x.at[0])
        xb_cp = pltpu.make_async_copy(bx_h, xb.at[1], sem_x.at[1])
        xa_cp.start()
        xb_cp.start()
        lax.fori_loop(1, S_W2 + lead, pro, 0)
        xa_cp.wait()
        xb_cp.wait()
        zeros = jnp.zeros((4, DM), F32)
        xa = jnp.concatenate([xb[0].astype(F32), zeros], axis=0).astype(BF)
        xq = jnp.concatenate([xb[1].astype(F32), zeros], axis=0).astype(BF)
        wait(bwqb, sem_w.at[0])
        wait(wukb, sem_w.at[1])
        s0 = S_W2 + lead

        def p1(i, c):
            issue(s0 + i, s0, s0 + 16)
            if do_compute:
                wq2 = head_pair(bwqb, i)
                wk2 = head_pair(wukb, i)
                for j in range(2):
                    q = _dot(xq, wq2[j]).astype(BF)
                    qa = _dot_nt(q, wk2[j])
                    r = pl.ds(pl.multiple_of((2 * i + j) * 8, 8), 8)
                    for n in range(4):
                        qabs_s[n, r, :] = qa[:, n * 128:(n + 1) * 128]
            return c
        lax.fori_loop(0, 16, p1, 0)
        wait(wqb, sem_w.at[2])
        wait(wuvb, sem_w.at[3])
        s1 = s0 + 16

        if do_compute:
            cc_s[...] = jnp.zeros(cc_s.shape, F32)

        def p2b(b, c):
            q = jnp.concatenate([qabs_s[n, pl.ds(b, H, stride=8), :] for n in range(4)], axis=1).astype(BF)

            def p2(j, carry):
                m, l, acc = carry
                t = b * 8 + j
                issue(s1 + t, s1, s1 + 32)
                blk = cb.at[pl.ds(pl.multiple_of(t * 512, 512), 512)]
                wait(blk, sem_c.at[j])
                if not do_compute:
                    return carry
                cblk = blk[...]
                s = _dot_nt(q, cblk) * SCALE
                m_new = jnp.maximum(m, jnp.max(s, axis=1, keepdims=True))
                alpha = jnp.exp(m - m_new)
                p = jnp.exp(s - m_new)
                l = alpha * l + jnp.sum(p, axis=1, keepdims=True)
                acc = alpha * acc + _dot(p.astype(BF), cblk)
                return m_new, l, acc
            m, l, acc = lax.fori_loop(
                0, 8, p2, (jnp.full((H, 1), -jnp.inf, F32), jnp.zeros((H, 1), F32), jnp.zeros((H, DC), F32)))
            if do_compute:
                cc = acc / l
                for n in range(4):
                    cc_s[n, pl.ds(b, H, stride=8), :] = cc[:, n * 128:(n + 1) * 128]
            return c
        lax.fori_loop(0, B, p2b, 0)
        s2 = s1 + 32

        def p3(i, c):
            issue(s2 + i, s2, s2 + 8)
            if do_compute:
                for u in range(2):
                    wv2 = head_pair(wuvb, 2 * i + u)
                    for j in range(2):
                        r = pl.ds(pl.multiple_of((4 * i + 2 * u + j) * 8, 8), 8)
                        cc = jnp.concatenate([cc_s[n, r, :] for n in range(4)], axis=1).astype(BF)
                        ctx_s[r, :] = _dot(cc, wv2[j])
                q = _dot(xa, wqb[:, pl.ds(pl.multiple_of(i * 512, 512), 512)])
                for n in range(4):
                    qa_s[pl.ds(pl.multiple_of((4 * i + n) * 8, 8), 8), :] = q[:, n * 128:(n + 1) * 128]
            return c
        lax.fori_loop(0, 8, p3, 0)
        s3 = s2 + 8

        if do_compute:
            o_s[...] = jnp.zeros(o_s.shape, F32)
        row = lax.broadcasted_iota(jnp.int32, (8, 128), 0)
        s4 = s3 + 15 * 8 + last_issue

        def p4(g, c):
            b = lax.shift_right_logical(g, 2)
            hg = (g & 3) * 8
            grp = pl.ds(pl.multiple_of(g * 8, 8), 8)
            wait(kb.at[grp], sem_kv.at[0, g & 1])
            wait(vb.at[grp], sem_kv.at[1, g & 1])
            q = qa_s[pl.ds(hg * 8 + b, 8, stride=8), :].astype(BF)

            def step(u):
                s = s3 + g * 8 + u
                pl.when(s < s4)(lambda: issue(s, s3, s4))

            def qk(u, c):
                step(u)
                if do_compute:
                    for j in range(2):
                        h = 2 * u + j
                        s = _dot_nt(q, kb[g * 8 + h])
                        for n in range(8):
                            pltpu.store(s_s.at[:, pl.ds(n * 128, 128)], s[:, n * 128:(n + 1) * 128], mask=row == h)
                return c
            lax.fori_loop(0, 4, qk, 0)
            s = s_s[...] * SCALE
            p = jnp.exp(s - jnp.max(s, axis=1, keepdims=True))
            l = jnp.sum(p, axis=1, keepdims=True)
            p = p.astype(BF)

            def pv(u, o):
                step(4 + u)
                if do_compute:
                    for j in range(2):
                        h = 2 * u + j
                        o = jnp.where(row == h, _dot(p, vb[g * 8 + h]), o)
                return o
            o = lax.fori_loop(0, 4, pv, jnp.zeros((8, DH), F32))
            if do_compute:
                o_s[pl.ds(hg * 8 + b, 8, stride=8), :] = o / l
            return c
        lax.fori_loop(0, 16, p4, 0)

        def p5(t, carry):
            ya, yb = carry
            pl.when(s4 + t < S_END)(lambda: issue(s4 + t, s4, S_END))
            r = pl.ds(pl.multiple_of(t * 256, 256), 256)
            wait(wob.at[r], sem_o.at[0, t])
            wait(bwob.at[r], sem_o.at[1, t])
            if not do_compute:
                return carry
            r0 = pl.ds(pl.multiple_of(t * 8, 8), 8)
            r1 = pl.ds(pl.multiple_of(t * 8 + 128, 8), 8)
            la = jnp.concatenate([o_s[r0, :], o_s[r1, :]], axis=1).astype(BF)
            lb = jnp.concatenate([ctx_s[r0, :], ctx_s[r1, :]], axis=1).astype(BF)
            return ya + _dot(la, wob[r, :]), yb + _dot(lb, bwob[r, :])
        ya, yb = lax.fori_loop(0, 16, p5, (jnp.zeros((8, DM), F32), jnp.zeros((8, DM), F32)))
        out_ref[:, 0:DM] = ya[0:4].astype(BF)
        out_ref[:, DM:2 * DM] = yb[0:4].astype(BF)

    def run(A_x, A_k_cache, A_v_cache, A_wq, A_wo, B_x, B_c_kv, B_w_q, B_w_uk, B_w_uv, B_w_o):
        vm = pltpu.VMEM
        dma = pltpu.SemaphoreType.DMA
        out = pl.pallas_call(
            kernel,
            out_shape=jax.ShapeDtypeStruct((B, 2 * DM), BF),
            in_specs=[pl.BlockSpec(memory_space=pltpu.HBM)] * 11,
            out_specs=pl.BlockSpec(memory_space=pltpu.VMEM),
            scratch_shapes=[
                vm((B * H, WIN, DH), BF), vm((B * H, WIN, DH), BF), vm((B * SK, DC), BF),
                vm((DM, H * DH), BF), vm((H * DH, DM), BF),
                vm((DM * H // 2, DH), jnp.uint32), vm((DC * H // 2, DH), jnp.uint32), vm((DC * H // 2, DH), jnp.uint32), vm((H * DH, DM), BF),
                vm((2, B, DM), BF),
                vm((H * 8, DH), F32), vm((4, H * 8, 128), F32), vm((4, H * 8, 128), F32),
                vm((H * 8, DH), F32), vm((H * 8, DH), F32), vm((8, WIN), F32),
                dma((2,)), dma((4,)), dma((8,)), dma((2, 2)), dma((2, 16)),
            ],
            compiler_params=pltpu.CompilerParams(
                vmem_limit_bytes=120 * 1024 * 1024, disable_bounds_checks=True),
        )(A_x.reshape(B, DM), A_k_cache.reshape(B * H, SK, DH), A_v_cache.reshape(B * H, SK, DH),
          A_wq, A_wo, B_x.reshape(B, DM), B_c_kv.reshape(B * SK, DC),
          B_w_q.reshape(DM * H, DH), B_w_uk.reshape(DC * H, DH), B_w_uv.reshape(DC * H, DH),
          B_w_o.reshape(H * DH, DM))
        return out.reshape(B, 1, 2 * DM)

    return run


@jax.jit
def pallas_concat_heads__sliding_block_cached__compressed_kv_cla__decode_kernel(
    A_x, A_k_cache, A_v_cache, A_wq, A_wo, B_x, B_c_kv, B_w_q, B_w_uk, B_w_uv, B_w_o,
):
    return make_kernel()(A_x, A_k_cache, A_v_cache, A_wq, A_wo, B_x, B_c_kv, B_w_q, B_w_uk, B_w_uv, B_w_o)
```

```python
import functools

import jax
import jax.numpy as jnp
from jax import lax
import jax.experimental.pallas as pl
import jax.experimental.pallas.tpu as pltpu

B, H, DH, DM, SK, WIN, DC = 4, 32, 128, 512, 4096, 1024, 512
BF, F32, U32 = jnp.bfloat16, jnp.float32, jnp.uint32
NT = (((1,), (1,)), ((), ()))
SCALE = DH ** -0.5

U_W1, U_C, U_W2, U_KV, U_WO, U_END = 0, 64, 192, 256, 768, 832
N_Q, N_C, N_X, N_A, N_O, N_END = 0, 16, 48, 64, 192, 224


def _dot(a, b):
    return jnp.dot(a, b, preferred_element_type=F32)


def _dot_nt(a, b):
    return lax.dot_general(a, b, NT, preferred_element_type=F32)


def _rows(piece, n):
    return pl.ds(pl.multiple_of(piece * n, n), n)


def _scatter_bits(u, bits):
    out, j = 0, 0
    while j < len(bits):
        n = 1
        while j + n < len(bits) and bits[j + n] == bits[j] + n:
            n += 1
        out = out + (((u >> j) & ((1 << n) - 1)) << bits[j])
        j += n
    return out


def make_kernel(do_dma=True, do_compute=True, pr="00110011", pad=1, wbits=(5, 0, 1, 2, 3, 4), wperm=(0, 1, 2, 3),
                cbits=(6, 0, 1, 2, 3, 4, 5), kvbits=(4, 0, 1, 2, 3), lastw=56,
                lead=16, r_c=5.0, r_x=3.0, t_k=781, r_k=2.0, r_o=1.5):
    ST = 32 + pad
    fix = lambda n, r: (n * int(r * 64)) >> 6
    hi_q = lambda n: U_C + lead + fix(n, (U_W2 - U_C - lead) / 15 + 1 / 64)
    t_c = U_W2 + lead
    hi_c = lambda n: t_c + fix(n, r_c)
    t_x = hi_c(31)
    hi_x = lambda n: t_x + fix(n + 1, r_x)
    t_a = hi_x(15)
    hi_a1 = lambda n: t_a + fix(n + 1, (t_k - t_a) / 121 + 1 / 64)
    hi_a2 = lambda n: t_k + fix(n - 120, r_k)
    t_o = hi_a2(127)
    hi_o = lambda n: t_o + fix(n + 1, r_o)
    assert hi_q(15) >= U_W2 and t_x >= U_KV + 10
    for g in range(16):
        assert min(hi_a1(8 * g), hi_a2(8 * g)) >= U_KV + 32 * (g + 1) + 8, g
    assert min(hi_a1(127), hi_a2(127)) == t_o
    for n in range(32):
        assert hi_o(n) >= min(U_WO + 8 * (n // 4 + 1) + 8, U_END), n

    def kernel(ax_h, k_h, v_h, wq_h, wo_h, bx_h, c_h, bwq_h, wuk_h, wuv_h, bwo_h, out_ref,
               kb, vb, cb, wqb, wob, bwqb, wukb, wuvb, bwob, xb,
               qa_s, qabs_s, cc_s, ctx_s, o_s, s_s, p_s, l_s, m_s, lc_s, acc_s, y_s,
               sem_x, sem_w, sem_c, sem_kv, sem_o):

        def burst(desc):
            cnt = [0, 0]
            for ch in pr:
                p = int(ch)
                src, dst, sem = desc(p, cnt[p])
                cnt[p] += 1
                pltpu.make_async_copy(src, dst, sem).start(priority=p)

        def head_major(src, dst, sem, x, i):
            return src.bitcast(U32).at[i, _rows(x, 32)], dst.at[pl.ds(x * ST + i * 64 * ST, 32)], sem

        def issue_w1(u):
            x = _scatter_bits(u, wbits)
            burst(lambda p, i: head_major((bwq_h, wuk_h)[p], (bwqb, wukb)[p], sem_w.at[p], x, wperm[i]))

        def issue_w2(u):
            x = _scatter_bits(u, wbits)
            r, cc = _rows(x >> 2, 8), _rows(x & 3, 1024)
            burst(lambda p, i: head_major(wuv_h, wuvb, sem_w.at[3], x, wperm[i]) if p else
                  (wq_h.at[wperm[i], r, cc], wqb.at[wperm[i], r, cc], sem_w.at[2]))

        def issue_c(u):
            x = _scatter_bits(u, cbits)
            b, r = x >> 6, _rows(x & 63, 16)
            burst(lambda p, i: (c_h.at[p, b, i, r], cb.at[p, b, i, r], sem_c.at[p]))

        def issue_kv(u):
            x = _scatter_bits(u, kvbits)
            g = u >> 5
            hq = g * 2 + (x >> 4)
            rs, rd = _rows((x & 15) + 48, 64), _rows(x & 15, 64)
            burst(lambda p, i: ((k_h, v_h)[p].at[hq, i, rs], (kb, vb)[p].at[hq, i, rd], sem_kv.at[p, g]))

        def issue_wo(u):
            last = u >= lastw
            x0 = jnp.where(last, (u & ~7) + (u & 1) * 4 + ((u >> 1) & 3) * 64, u)
            dx = jnp.where(last, 1, 64)

            def desc(p, i):
                x = x0 + i * dx
                return (wo_h, bwo_h)[p].at[_rows(x, 16)], (wob, bwob)[p].at[_rows(x, 16)], sem_o.at[p, x >> 3]
            burst(desc)

        W1, CC, W2 = (U_W1, U_C, issue_w1), (U_C, U_W2, issue_c), (U_W2, U_KV, issue_w2)
        KV, WO = (U_KV, U_WO, issue_kv), (U_WO, U_END, issue_wo)

        def phase(count, unit, start, target, *streams):
            def body(n, done):
                hi = target(n)
                if do_dma:
                    for a, e, f in streams:
                        pl.loop(jnp.maximum(done - a, 0), jnp.minimum(hi, e) - a)(f)
                unit(n)
                return hi
            lax.fori_loop(0, count, body, start)

        def wait(ref, sem):
            if do_dma:
                pltpu.make_async_copy(ref, ref, sem).wait()

        def head_pair(w_ref, i):
            ev = w_ref[pl.ds(i, 256, stride=ST), :]
            od = w_ref[pl.ds(i + 16, 256, stride=ST), :]
            lo = (ev & jnp.uint32(0xFFFF)) | (od << 16)
            hi = (ev >> 16) | (od & jnp.uint32(0xFFFF0000))
            return pltpu.bitcast(lo, BF), pltpu.bitcast(hi, BF)

        def x_rows(n):
            return jnp.concatenate([xb[n].astype(F32), jnp.zeros((4, DM), F32)], axis=0).astype(BF)

        xa_cp = pltpu.make_async_copy(ax_h, xb.at[0], sem_x.at[0])
        xb_cp = pltpu.make_async_copy(bx_h, xb.at[1], sem_x.at[1])

        def unit_q(i):
            @pl.when(i == 0)
            def _():
                xa_cp.wait()
                xb_cp.wait()
                wait(bwqb.at[pl.ds(0, 8192)], sem_w.at[0])
                wait(wukb.at[pl.ds(0, 8192)], sem_w.at[1])
            if not do_compute:
                return
            xq = x_rows(1)
            wq2 = head_pair(bwqb, i)
            wk2 = head_pair(wukb, i)
            for j in range(2):
                q = _dot(xq, wq2[j]).astype(BF)
                qa = _dot_nt(q, wk2[j])
                r = _rows(2 * i + j, 8)
                for n in range(4):
                    qabs_s[n, r, :] = qa[:, n * 128:(n + 1) * 128]
                    cc_s[n, r, :] = jnp.zeros((8, 128), F32)
                o_s[r, :] = jnp.zeros((8, 128), F32)

        def unit_c(t):
            b, j = t >> 3, t & 7

            @pl.when(t == 0)
            def _():
                wait(cb.at[0], sem_c.at[0])
                wait(cb.at[1], sem_c.at[1])
            if not do_compute:
                return

            @pl.when(j == 0)
            def _():
                m_s[...] = jnp.full(m_s.shape, -jnp.inf, F32)
                lc_s[...] = jnp.zeros(lc_s.shape, F32)
                acc_s[...] = jnp.zeros(acc_s.shape, F32)
            q = jnp.concatenate([qabs_s[n, pl.ds(b, H, stride=8), :] for n in range(4)], axis=1).astype(BF)
            cblk = cb[b >> 1, b & 1, j >> 1, _rows(j & 1, 512), :]
            s = _dot_nt(q, cblk) * SCALE
            m = m_s[...]
            m_new = jnp.maximum(m, jnp.max(s, axis=1, keepdims=True))
            alpha = jnp.exp(m - m_new)
            p = [jnp.exp(s[:, n * 128:(n + 1) * 128] - m_new) for n in range(4)]
            m_s[...] = m_new
            lc_s[...] = alpha * lc_s[...] + ((p[0] + p[1]) + (p[2] + p[3]))
            pv = _dot(jnp.concatenate(p, axis=1).astype(BF), cblk)
            for n in range(4):
                acc_s[n] = alpha * acc_s[n] + pv[:, n * 128:(n + 1) * 128]

            @pl.when(j == 7)
            def _():
                l = jnp.sum(lc_s[...], axis=1, keepdims=True)
                for n in range(4):
                    cc_s[n, pl.ds(b, H, stride=8), :] = acc_s[n] / l

        def unit_x(i):
            @pl.when(i == 0)
            def _():
                wait(wqb, sem_w.at[2])
                wait(wuvb.at[pl.ds(0, 8192)], sem_w.at[3])
            if not do_compute:
                return
            wv2 = head_pair(wuvb, i)
            for j in range(2):
                r = _rows(2 * i + j, 8)
                cc = jnp.concatenate([cc_s[n, r, :] for n in range(4)], axis=1).astype(BF)
                ctx_s[r, :] = _dot(cc, wv2[j])
            q = _dot(x_rows(0), wqb[:, :, _rows(i, 256)].reshape(DM, 256))
            for j in range(2):
                qa_s[_rows(2 * i + j, 8), :] = q[:, j * 128:(j + 1) * 128]

        def unit_a(n):
            g, u = n >> 3, n & 7
            mine = pl.ds((g & 3) * 64 + (g >> 2), 8, stride=8)
            row = lax.broadcasted_iota(jnp.int32, (8, 128), 0)
            hq, hi = g * 2 + ((u >> 1) & 1), (u & 1) * 2

            @pl.when(u == 0)
            def _():
                wait(kb.at[pl.ds(g * 2, 2)], sem_kv.at[0, g])
                wait(vb.at[pl.ds(g * 2, 2)], sem_kv.at[1, g])
            if not do_compute:
                return

            @pl.when(u < 4)
            def _():
                q = qa_s[mine, :].astype(BF)
                for j in range(2):
                    s = _dot_nt(q, kb[hq, hi + j])
                    for m in range(8):
                        pltpu.store(s_s.at[:, pl.ds(m * 128, 128)], s[:, m * 128:(m + 1) * 128],
                                    mask=row == 2 * u + j)

            @pl.when(u == 3)
            def _():
                s = s_s[...] * SCALE
                p = jnp.exp(s - jnp.max(s, axis=1, keepdims=True))
                l_s[...] = jnp.broadcast_to(jnp.sum(p, axis=1, keepdims=True), l_s.shape)
                p_s[...] = p

            @pl.when(u >= 4)
            def _():
                p = p_s[...].astype(BF)
                o = o_s[mine, :]
                for j in range(2):
                    o = jnp.where(row == 2 * (u - 4) + j, _dot(p, vb[hq, hi + j]) / l_s[...], o)
                o_s[mine, :] = o

        def unit_o(n):
            h = (n >> 2) + 8 * (n & 3)
            r = _rows(h, 128)
            wait(wob.at[r], sem_o.at[0, h])
            wait(bwob.at[r], sem_o.at[1, h])
            if not do_compute:
                out_ref[...] = jnp.zeros(out_ref.shape, BF)
                return
            for m, (a_s, w) in enumerate(((o_s, wob), (ctx_s, bwob))):
                y = y_s[m] + _dot(a_s[_rows(h, 8), :].astype(BF), w[r, :])
                y_s[m] = y
                out_ref[:, m * DM:(m + 1) * DM] = y[0:4].astype(BF)

        if do_dma:
            @pl.loop(0, U_C)
            def _(u):
                issue_w1(u)

                @pl.when(u == 7)
                def _():
                    xa_cp.start()
                    xb_cp.start(priority=1)
        else:
            xa_cp.start()
            xb_cp.start(priority=1)
        y_s[...] = jnp.zeros(y_s.shape, F32)
        phase(16, unit_q, U_C, hi_q, CC)
        phase(32, unit_c, U_W2, hi_c, W2, KV)
        phase(16, unit_x, t_x, hi_x, KV)
        phase(128, unit_a, t_a, lambda n: jnp.minimum(hi_a1(n), hi_a2(n)), KV, WO)
        phase(32, unit_o, t_o, hi_o, WO)

    def run(A_x, A_k_cache, A_v_cache, A_wq, A_wo, B_x, B_c_kv, B_w_q, B_w_uk, B_w_uv, B_w_o):
        vm = pltpu.VMEM
        dma = pltpu.SemaphoreType.DMA
        out = pl.pallas_call(
            kernel,
            out_shape=jax.ShapeDtypeStruct((B, 2 * DM), BF),
            in_specs=[pl.BlockSpec(memory_space=pltpu.HBM)] * 11,
            out_specs=pl.BlockSpec(memory_space=pltpu.VMEM),
            scratch_shapes=[
                vm((32, 4, WIN, DH), BF), vm((32, 4, WIN, DH), BF), vm((2, 2, 4, 1024, DC), BF),
                vm((4, 128, H * DH), BF), vm((H * DH, DM), BF),
                vm((256 * ST, DH), U32), vm((256 * ST, DH), U32), vm((256 * ST, DH), U32), vm((H * DH, DM), BF),
                vm((2, B, DM), BF),
                vm((H * 8, DH), F32), vm((4, H * 8, 128), F32), vm((4, H * 8, 128), F32),
                vm((H * 8, DH), F32), vm((H * 8, DH), F32), vm((8, WIN), F32), vm((8, WIN), F32), vm((8, 128), F32),
                vm((H, 128), F32), vm((H, 128), F32), vm((4, H, 128), F32), vm((2, 8, DM), F32),
                dma((2,)), dma((4,)), dma((2,)), dma((2, 16)), dma((2, 32)),
            ],
            compiler_params=pltpu.CompilerParams(
                vmem_limit_bytes=120 * 1024 * 1024, disable_bounds_checks=True, disable_semaphore_checks=True),
        )(A_x.reshape(B, DM), A_k_cache.reshape(32, 4, SK, DH), A_v_cache.reshape(32, 4, SK, DH),
          A_wq.reshape(4, 128, H * DH), A_wo, B_x.reshape(B, DM), B_c_kv.reshape(2, 2, 4, 1024, DC),
          B_w_q.reshape(4, 4096, DH), B_w_uk.reshape(4, 4096, DH), B_w_uv.reshape(4, 4096, DH),
          B_w_o.reshape(H * DH, DM))
        return out.reshape(B, 1, 2 * DM)

    return run


@jax.jit
def pallas_concat_heads__sliding_block_cached__compressed_kv_cla__decode_kernel(
    A_x, A_k_cache, A_v_cache, A_wq, A_wo, B_x, B_c_kv, B_w_q, B_w_uk, B_w_uv, B_w_o,
):
    return make_kernel(pad=0)(A_x, A_k_cache, A_v_cache, A_wq, A_wo, B_x, B_c_kv, B_w_q, B_w_uk, B_w_uv, B_w_o)
```

```python
import jax
import jax.numpy as jnp
from jax import lax
import jax.experimental.pallas as pl
import jax.experimental.pallas.tpu as pltpu

B, H, DH, DM, SK, DC = 4, 32, 128, 512, 4096, 512
WIN = min(4096, max(256, SK // 4))
SCALE = DH ** -0.5
BF16, F32, U32 = jnp.bfloat16, jnp.float32, jnp.uint32

QUEUES = (0, 0, 1, 1, 0, 0, 1, 1)
W1, CKV, W2, KV, WO, LAST, END = 0, 64, 192, 256, 768, 824, 832
PITCH = H + 1


def _dot(a, b):
    return jnp.dot(a, b, preferred_element_type=F32)


def _dot_nt(a, b):
    return lax.dot_general(a, b, (((1,), (1,)), ((), ())), preferred_element_type=F32)


def _block(i, n):
    return pl.ds(i * n if isinstance(i, int) else pl.multiple_of(i * n, n), n)


def _lanes(x, n):
    return x[:, n * 128:(n + 1) * 128]


def _ramp(start, rate):
    return lambda n: start + ((n * int(rate * 64)) >> 6)


_query_at = _ramp(CKV + 16, 4.9)
_latent_at = _ramp(W2 + 16, 5)
_regroup_at = _ramp(_latent_at(31) + 2, 2)
_context_at = _ramp(_regroup_at(3) + 2, 2.5)
_window_early, _window_late = _ramp(_context_at(15) + 3, 3.08), _ramp(781 - 240, 2)
_output_at = _ramp(_window_late(127) + 6, 6)
assert _query_at(23) >= W2 and _regroup_at(0) >= KV + 8 and _context_at(15) <= WO
assert all(min(_window_early(8 * g), _window_late(8 * g)) >= KV + 32 * (g + 1) + 8 for g in range(16))
assert _window_late(127) <= min(_window_early(127), LAST)
assert all(_output_at(n) >= WO + 8 * (n + 1) + 8 for n in range(7)) and _output_at(6) >= END


def _kernel(ax_h, k_h, v_h, wq_h, wo_h, bx_h, c_h, bwq_h, wuk_h, wuv_h, bwo_h, out_ref,
            kb, vb, cb, wqb, wob, bwqb, wukb, wuvb, xb, heads0, heads1,
            qa_s, qc_s, cc_s, o_s, s_s, p_s, l_s, m_s, lc_s, acc_s, y_s,
            sem_x, sem_w, sem_c, sem_kv, sem_o):

    def burst(copy):
        count = [0, 0]
        for q in QUEUES:
            pltpu.make_async_copy(*copy(q, count[q])).start(priority=q)
            count[q] += 1

    def weight_piece(u):
        return (u >> 1) + (u & 1) * 32

    def issue_w1(u):
        r = _block(weight_piece(u), 64)
        burst(lambda q, i: ((bwq_h, wuk_h)[q].at[i, r], (bwqb, wukb)[q].at[i, r], sem_w.at[q]))

    def issue_ckv(u):
        b, r = u & 1, _block(u >> 1, 16)
        burst(lambda q, i: (c_h.at[q, b, i, r], cb.at[q, b, i, r], sem_c))

    def issue_w2(u):
        x = weight_piece(u)
        r, rq, cq = _block(x, 64), _block(x >> 2, 8), _block(x & 3, 1024)
        burst(lambda q, i: (wuv_h.at[i, r], wuvb.at[i, r], sem_w.at[3]) if q else
              (wq_h.at[i, rq, cq], wqb.at[i, rq, cq], sem_w.at[2]))

    def issue_kv(u):
        g, x = u >> 5, (u >> 1) & 15
        hq = 2 * g + (u & 1)
        src, dst = _block(x + (SK - WIN) // 64, 64), _block(x, 64)
        burst(lambda q, i: ((k_h, v_h)[q].at[hq, i, src], (kb, vb)[q].at[hq, i, dst], sem_kv.at[q, g]))

    def issue_wo(u):
        r = _block(u, 16)
        burst(lambda q, i: ((wo_h, bwo_h)[q].at[i, r], wob.at[q, i, r], sem_o.at[u >> 3]))

    def issue_last(u):
        i, x = u >> 1, 56 + 4 * (u & 1)
        burst(lambda q, j: ((wo_h, bwo_h)[q].at[i, _block(x + j, 16)], wob.at[q, i, _block(x + j, 16)],
                            sem_o.at[7 + i]))

    def issue(first, last, fn):
        def run(done, target):
            pl.loop(jnp.maximum(done - first, 0), jnp.minimum(target, last) - first)(fn)
        return run

    def phase(count, unit, done, target, *streams):
        def body(n, done):
            for stream in streams:
                stream(done, target(n))
            unit(n)
            return target(n)
        lax.fori_loop(0, count, body, done)

    def wait(ref, sem):
        pltpu.make_async_copy(ref, ref, sem).wait()

    x_copies = [pltpu.make_async_copy(x, xb.at[n], sem_x.at[n]) for n, x in enumerate((ax_h, bx_h))]

    def x_rows(n):
        return jnp.concatenate([xb[n].astype(F32), jnp.zeros((8 - B, DM), F32)], axis=0).astype(BF16)

    def regroup(src, dst, i):
        for j in range(32):
            w = pltpu.bitcast(src[i >> 1, _block((i & 1) * 32 + j, 64), :], U32)
            row0, row1 = w[:16], w[16:]
            even = (row0 & jnp.uint32(0xFFFF)) | (row1 << 16)
            odd = (row0 >> 16) | (row1 & jnp.uint32(0xFFFF0000))
            dst[pl.ds((i * 32 + j) * PITCH, H), :] = jnp.concatenate([even, odd], axis=0)

    def head(w_ref, pair, j):
        return pltpu.bitcast(w_ref[pl.ds(pair + 16 * j, 256, stride=PITCH), :], BF16)

    def unit_query(n):
        @pl.when(n == 0)
        def _():
            for copy in x_copies:
                copy.wait()
            wait(bwqb, sem_w.at[0])
            wait(wukb, sem_w.at[1])

        @pl.when(n < 8)
        def _():
            regroup(bwqb, heads0, n)
            regroup(wukb, heads1, n)

        @pl.when(n >= 8)
        def _():
            x = x_rows(1)
            for j in range(2):
                q = _dot(x, head(heads0, n - 8, j)).astype(BF16)
                qc = _dot_nt(q, head(heads1, n - 8, j))
                r = _block(2 * (n - 8) + j, 8)
                for k in range(4):
                    qc_s[k, r, :] = _lanes(qc, k)
                    cc_s[k, r, :] = jnp.zeros((8, 128), F32)
                o_s[0, r, :] = jnp.zeros((8, 128), F32)

    def unit_latent(n):
        b, j = n >> 3, n & 7
        heads = pl.ds(b, H, stride=8)
        pl.when(n == 0)(lambda: wait(cb, sem_c))

        @pl.when(j == 0)
        def _():
            m_s[...] = jnp.full(m_s.shape, -jnp.inf, F32)
            lc_s[...] = jnp.zeros(lc_s.shape, F32)
            acc_s[...] = jnp.zeros(acc_s.shape, F32)
        q = jnp.concatenate([qc_s[k, heads, :] for k in range(4)], axis=1).astype(BF16)
        c = cb[b >> 1, b & 1, j >> 1, _block(j & 1, 512), :]
        s = _dot_nt(q, c) * SCALE
        m_old = m_s[...]
        m_new = jnp.maximum(m_old, jnp.max(s, axis=1, keepdims=True))
        alpha = jnp.exp(m_old - m_new)
        p = [jnp.exp(_lanes(s, k) - m_new) for k in range(4)]
        m_s[...] = m_new
        lc_s[...] = alpha * lc_s[...] + ((p[0] + p[1]) + (p[2] + p[3]))
        pc = _dot(jnp.concatenate(p, axis=1).astype(BF16), c)
        for k in range(4):
            acc_s[k] = alpha * acc_s[k] + _lanes(pc, k)

        @pl.when(j == 7)
        def _():
            l = jnp.sum(lc_s[...], axis=1, keepdims=True)
            for k in range(4):
                cc_s[k, heads, :] = acc_s[k] / l

    def unit_regroup(n):
        @pl.when(n == 0)
        def _():
            wait(wqb, sem_w.at[2])
            wait(wuvb, sem_w.at[3])
        regroup(wuvb, heads0, 2 * n)
        regroup(wuvb, heads0, 2 * n + 1)

    def unit_context(n):
        q = _dot(x_rows(0), wqb[:, :, _block(n, 256)].reshape(DM, 256))
        for j in range(2):
            r = _block(2 * n + j, 8)
            cc = jnp.concatenate([cc_s[k, r, :] for k in range(4)], axis=1).astype(BF16)
            o_s[1, r, :] = _dot(cc, head(heads0, n, j))
            qa_s[r, :] = _lanes(q, j)

    def unit_window(n):
        g, u = n >> 3, n & 7
        heads = pl.ds((g & 3) * 64 + (g >> 2), 8, stride=8)
        hq, hi = 2 * g + ((u >> 1) & 1), (u & 1) * 2

        @pl.when(u == 0)
        def _():
            wait(kb.at[pl.ds(2 * g, 2)], sem_kv.at[0, g])
            wait(vb.at[pl.ds(2 * g, 2)], sem_kv.at[1, g])

        @pl.when(u < 4)
        def _():
            q = qa_s[heads, :].astype(BF16)
            row = lax.broadcasted_iota(jnp.int32, (8, WIN), 0)
            s = s_s[...]
            for j in range(2):
                s = jnp.where(row == 2 * u + j, _dot_nt(q, kb[hq, hi + j]), s)
            s_s[...] = s

        @pl.when(u == 3)
        def _():
            s = s_s[...] * SCALE
            p = jnp.exp(s - jnp.max(s, axis=1, keepdims=True))
            l_s[...] = jnp.broadcast_to(jnp.sum(p, axis=1, keepdims=True), l_s.shape)
            p_s[...] = p

        @pl.when(u >= 4)
        def _():
            p = p_s[...].astype(BF16)
            row = lax.broadcasted_iota(jnp.int32, (8, DH), 0)
            o = o_s[0, heads, :]
            for j in range(2):
                o = jnp.where(row == 2 * (u - 4) + j, _dot(p, vb[hq, hi + j]) / l_s[...], o)
            o_s[0, heads, :] = o

    def project(m, i, n):
        return _dot(o_s[m, _block(8 * i + n, 8), :].astype(BF16), wob[m, i, _block(n, 128), :])

    def unit_output(n):
        wait(wob.at[:, :, _block(n, 128)], sem_o.at[n])
        for m in range(2):
            y_s[m] += (project(m, 0, n) + project(m, 1, n)) + (project(m, 2, n) + project(m, 3, n))

    @pl.loop(W1, CKV)
    def _(u):
        issue_w1(u)

        @pl.when(u == 7)
        def _():
            for n, copy in enumerate(x_copies):
                copy.start(priority=n)

    y_s[...] = jnp.zeros(y_s.shape, F32)
    s_s[...] = jnp.zeros(s_s.shape, F32)
    kv, wo = issue(KV, WO, issue_kv), issue(WO, LAST, issue_wo)
    phase(24, unit_query, CKV, _query_at, issue(CKV, W2, issue_ckv))
    phase(32, unit_latent, W2, _latent_at, issue(W2, KV, issue_w2), kv)
    phase(4, unit_regroup, _latent_at(31), _regroup_at, kv)
    phase(16, unit_context, _regroup_at(3), _context_at, kv)
    phase(128, unit_window, _context_at(15),
          lambda n: jnp.minimum(_window_early(n), _window_late(n)), kv, wo)
    phase(7, unit_output, _window_late(127), _output_at, wo, issue(LAST, END, issue_last))

    @pl.loop(0, 4)
    def _(i):
        wait(wob.at[:, i, _block(7, 128)], sem_o.at[7 + i])
        for m in range(2):
            y = y_s[m] + project(m, i, 7)
            y_s[m] = y
            out_ref[:, _block(m, DM)] = y[:B].astype(BF16)


@jax.jit
def pallas_concat_heads__sliding_block_cached__compressed_kv_cla__decode_kernel(
    A_x, A_k_cache, A_v_cache, A_wq, A_wo, B_x, B_c_kv, B_w_q, B_w_uk, B_w_uv, B_w_o,
):
    vmem, dma = pltpu.VMEM, pltpu.SemaphoreType.DMA
    per_head = H * 8 + 8
    out = pl.pallas_call(
        _kernel,
        out_shape=jax.ShapeDtypeStruct((B, 2 * DM), BF16),
        in_specs=[pl.BlockSpec(memory_space=pltpu.HBM)] * 11,
        out_specs=pl.BlockSpec(memory_space=pltpu.VMEM),
        scratch_shapes=[
            vmem((32, 4, WIN, DH), BF16), vmem((32, 4, WIN, DH), BF16), vmem((2, 2, 4, SK // 4, DC), BF16),
            vmem((4, DM // 4, H * DH), BF16), vmem((2, 4, 8 * DH, DM), BF16),
            vmem((4, 128 * H, DH), BF16), vmem((4, 128 * H, DH), BF16), vmem((4, 128 * H, DH), BF16),
            vmem((2, B, DM), BF16),
            vmem((257 * PITCH + 7, DH), U32), vmem((257 * PITCH + 7, DH), U32),
            vmem((per_head, DH), F32), vmem((4, per_head, 128), F32), vmem((4, per_head, 128), F32),
            vmem((2, per_head, DH), F32),
            vmem((8, WIN), F32), vmem((8, WIN), F32), vmem((8, 128), F32),
            vmem((H, 128), F32), vmem((H, 128), F32), vmem((4, H, 128), F32), vmem((2, 8, DM), F32),
            dma((2,)), dma((4,)), dma, dma((2, 16)), dma((11,)),
        ],
        compiler_params=pltpu.CompilerParams(
            vmem_limit_bytes=120 * 1024 * 1024,
            disable_bounds_checks=True,
            disable_semaphore_checks=True,
        ),
    )(
        A_x.reshape(B, DM), A_k_cache.reshape(32, 4, SK, DH), A_v_cache.reshape(32, 4, SK, DH),
        A_wq.reshape(4, DM // 4, H * DH), A_wo.reshape(4, 8 * DH, DM),
        B_x.reshape(B, DM), B_c_kv.reshape(2, 2, 4, SK // 4, DC),
        B_w_q.reshape(4, 128 * H, DH), B_w_uk.reshape(4, 128 * H, DH), B_w_uv.reshape(4, 128 * H, DH),
        B_w_o.reshape(4, 8 * DH, DM),
    )
    return out.reshape(B, 1, 2 * DM)
```

```python
import jax
import jax.numpy as jnp
from jax import lax
import jax.experimental.pallas as pl
import jax.experimental.pallas.tpu as pltpu

B, H, DH, DM, SK, DC = 4, 32, 128, 512, 4096, 512
WIN = min(4096, max(256, SK // 4))
SCALE = DH ** -0.5
BF16, F32, U32 = jnp.bfloat16, jnp.float32, jnp.uint32

QUEUES = (0, 0, 1, 1, 0, 0, 1, 1)
W1, CKV, W2, KV, WO, LAST, END = 0, 64, 192, 256, 768, 824, 832
PITCH = H + 1


def _dot(a, b):
    return jnp.dot(a, b, preferred_element_type=F32)


def _dot_nt(a, b):
    return lax.dot_general(a, b, (((1,), (1,)), ((), ())), preferred_element_type=F32)


def _block(i, n):
    return pl.ds(i * n if isinstance(i, int) else pl.multiple_of(i * n, n), n)


def _lanes(x, n):
    return x[:, n * 128:(n + 1) * 128]


def _ramp(start, rate):
    return lambda n: start + ((n * int(rate * 64)) >> 6)


_query_at = _ramp(CKV + 16, 4.9)
_latent_at = _ramp(W2 + 16, 5)
_regroup_at = _ramp(_latent_at(31) + 2, 2)
_context_at = _ramp(_regroup_at(3) + 2, 2.5)
_window_early, _window_late = _ramp(_context_at(15) + 3, 3.08), _ramp(781 - 240, 2)
_output_at = _ramp(_window_late(127) + 6, 6)
assert _query_at(23) >= W2 and _regroup_at(0) >= KV + 8 and _context_at(15) <= WO
assert all(min(_window_early(8 * g), _window_late(8 * g)) >= KV + 32 * (g + 1) + 8 for g in range(16))
assert _window_late(127) <= min(_window_early(127), LAST)
assert all(_output_at(n) >= WO + 8 * (n + 1) + 8 for n in range(7)) and _output_at(6) >= END


def _kernel(ax_h, k_h, v_h, wq_h, wo_h, bx_h, c_h, bwq_h, wuk_h, wuv_h, bwo_h, out_ref,
            kb, vb, cb, wqb, wob, bwqb, wukb, wuvb, xb, heads0, heads1,
            qa_s, qc_s, cc_s, o_s, s_s, p_s, l_s, m_s, lc_s, acc_s, y_s,
            sem_x, sem_w, sem_c, sem_kv, sem_o):

    def burst(copy):
        count = [0, 0]
        for q in QUEUES:
            pltpu.make_async_copy(*copy(q, count[q])).start(priority=q)
            count[q] += 1

    def issue_w1(u):
        r = _block(u, 64)
        burst(lambda q, i: ((bwq_h, wuk_h)[q].at[i, r], (bwqb, wukb)[q].at[i, r], sem_w.at[q]))

    def issue_ckv(u):
        b, r = u & 1, _block(u >> 1, 16)
        burst(lambda q, i: (c_h.at[q, b, i, r], cb.at[q, b, i, r], sem_c))

    def issue_w2(u):
        r, rq, cq = _block(u, 64), _block(u >> 2, 8), _block(u & 3, 1024)
        burst(lambda q, i: (wuv_h.at[i, r], wuvb.at[i, r], sem_w.at[3]) if q else
              (wq_h.at[i, rq, cq], wqb.at[i, rq, cq], sem_w.at[2]))

    def issue_kv(u):
        g, x = u >> 5, (u >> 1) & 15
        hq = 2 * g + (u & 1)
        src, dst = _block(x + (SK - WIN) // 64, 64), _block(x, 64)
        burst(lambda q, i: ((k_h, v_h)[q].at[hq, i, src], (kb, vb)[q].at[hq, i, dst], sem_kv.at[q, g]))

    def issue_wo(u):
        r = _block(u, 16)
        burst(lambda q, i: ((wo_h, bwo_h)[q].at[i, r], wob.at[q, i, r], sem_o.at[u >> 3]))

    def issue_last(u):
        i, x = u >> 1, 56 + 4 * (u & 1)
        burst(lambda q, j: ((wo_h, bwo_h)[q].at[i, _block(x + j, 16)], wob.at[q, i, _block(x + j, 16)],
                            sem_o.at[7 + i]))

    def issue(first, last, fn):
        def run(done, target):
            pl.loop(jnp.maximum(done - first, 0), jnp.minimum(target, last) - first)(fn)
        return run

    def phase(count, unit, done, target, *streams):
        def body(n, done):
            for stream in streams:
                stream(done, target(n))
            unit(n)
            return target(n)
        lax.fori_loop(0, count, body, done)

    def wait(ref, sem):
        pltpu.make_async_copy(ref, ref, sem).wait()

    x_copies = [pltpu.make_async_copy(x, xb.at[n], sem_x.at[n]) for n, x in enumerate((ax_h, bx_h))]

    def x_rows(n):
        return jnp.concatenate([xb[n].astype(F32), jnp.zeros((8 - B, DM), F32)], axis=0).astype(BF16)

    def regroup(src, dst, i):
        for j in range(32):
            w = pltpu.bitcast(src[i >> 1, _block((i & 1) * 32 + j, 64), :], U32)
            row0, row1 = w[:16], w[16:]
            even = (row0 & jnp.uint32(0xFFFF)) | (row1 << 16)
            odd = (row0 >> 16) | (row1 & jnp.uint32(0xFFFF0000))
            dst[pl.ds((i * 32 + j) * PITCH, H), :] = jnp.concatenate([even, odd], axis=0)

    def head(w_ref, pair, j):
        return pltpu.bitcast(w_ref[pl.ds(pair + 16 * j, 256, stride=PITCH), :], BF16)

    def unit_query(n):
        @pl.when(n == 0)
        def _():
            for copy in x_copies:
                copy.wait()
            wait(bwqb, sem_w.at[0])
            wait(wukb, sem_w.at[1])

        @pl.when(n < 8)
        def _():
            regroup(bwqb, heads0, n)
            regroup(wukb, heads1, n)

        @pl.when(n >= 8)
        def _():
            x = x_rows(1)
            for j in range(2):
                q = _dot(x, head(heads0, n - 8, j)).astype(BF16)
                qc = _dot_nt(q, head(heads1, n - 8, j))
                r = _block(2 * (n - 8) + j, 8)
                for k in range(4):
                    qc_s[k, r, :] = _lanes(qc, k)
                    cc_s[k, r, :] = jnp.zeros((8, 128), F32)
                o_s[0, r, :] = jnp.zeros((8, 128), F32)

    def unit_latent(n):
        b, j = n >> 3, n & 7
        heads = pl.ds(b, H, stride=8)
        pl.when(n == 0)(lambda: wait(cb, sem_c))

        @pl.when(j == 0)
        def _():
            m_s[...] = jnp.full(m_s.shape, -jnp.inf, F32)
            lc_s[...] = jnp.zeros(lc_s.shape, F32)
            acc_s[...] = jnp.zeros(acc_s.shape, F32)
        q = jnp.concatenate([qc_s[k, heads, :] for k in range(4)], axis=1).astype(BF16)
        c = cb[b >> 1, b & 1, j >> 1, _block(j & 1, 512), :]
        s = _dot_nt(q, c) * SCALE
        m_old = m_s[...]
        m_new = jnp.maximum(m_old, jnp.max(s, axis=1, keepdims=True))
        alpha = jnp.exp(m_old - m_new)
        p = [jnp.exp(_lanes(s, k) - m_new) for k in range(4)]
        m_s[...] = m_new
        lc_s[...] = alpha * lc_s[...] + ((p[0] + p[1]) + (p[2] + p[3]))
        pc = _dot(jnp.concatenate(p, axis=1).astype(BF16), c)
        for k in range(4):
            acc_s[k] = alpha * acc_s[k] + _lanes(pc, k)

        @pl.when(j == 7)
        def _():
            l = jnp.sum(lc_s[...], axis=1, keepdims=True)
            for k in range(4):
                cc_s[k, heads, :] = acc_s[k] / l

    def unit_regroup(n):
        @pl.when(n == 0)
        def _():
            wait(wqb, sem_w.at[2])
            wait(wuvb, sem_w.at[3])
        regroup(wuvb, heads0, 2 * n)
        regroup(wuvb, heads0, 2 * n + 1)

    def unit_context(n):
        q = _dot(x_rows(0), wqb[:, :, _block(n, 256)].reshape(DM, 256))
        for j in range(2):
            r = _block(2 * n + j, 8)
            cc = jnp.concatenate([cc_s[k, r, :] for k in range(4)], axis=1).astype(BF16)
            o_s[1, r, :] = _dot(cc, head(heads0, n, j))
            qa_s[r, :] = _lanes(q, j)

    def unit_window(n):
        g, u = n >> 3, n & 7
        heads = pl.ds((g & 3) * 64 + (g >> 2), 8, stride=8)
        hq, hi = 2 * g + ((u >> 1) & 1), (u & 1) * 2

        @pl.when(u == 0)
        def _():
            wait(kb.at[pl.ds(2 * g, 2)], sem_kv.at[0, g])
            wait(vb.at[pl.ds(2 * g, 2)], sem_kv.at[1, g])

        @pl.when(u < 4)
        def _():
            q = qa_s[heads, :].astype(BF16)
            row = lax.broadcasted_iota(jnp.int32, (8, WIN), 0)
            s = s_s[...]
            for j in range(2):
                s = jnp.where(row == 2 * u + j, _dot_nt(q, kb[hq, hi + j]), s)
            s_s[...] = s

        @pl.when(u == 3)
        def _():
            s = s_s[...] * SCALE
            p = jnp.exp(s - jnp.max(s, axis=1, keepdims=True))
            l_s[...] = jnp.broadcast_to(jnp.sum(p, axis=1, keepdims=True), l_s.shape)
            p_s[...] = p

        @pl.when(u >= 4)
        def _():
            p = p_s[...].astype(BF16)
            row = lax.broadcasted_iota(jnp.int32, (8, DH), 0)
            o = o_s[0, heads, :]
            for j in range(2):
                o = jnp.where(row == 2 * (u - 4) + j, _dot(p, vb[hq, hi + j]) / l_s[...], o)
            o_s[0, heads, :] = o

    def project(m, i, n):
        return _dot(o_s[m, _block(8 * i + n, 8), :].astype(BF16), wob[m, i, _block(n, 128), :])

    def unit_output(n):
        wait(wob.at[:, :, _block(n, 128)], sem_o.at[n])
        for m in range(2):
            y_s[m] += (project(m, 0, n) + project(m, 1, n)) + (project(m, 2, n) + project(m, 3, n))

    @pl.loop(W1, CKV)
    def _(u):
        issue_w1(u)

        @pl.when(u == 7)
        def _():
            for n, copy in enumerate(x_copies):
                copy.start(priority=n)

    y_s[...] = jnp.zeros(y_s.shape, F32)
    s_s[...] = jnp.zeros(s_s.shape, F32)
    kv, wo = issue(KV, WO, issue_kv), issue(WO, LAST, issue_wo)
    phase(24, unit_query, CKV, _query_at, issue(CKV, W2, issue_ckv))
    phase(32, unit_latent, W2, _latent_at, issue(W2, KV, issue_w2), kv)
    phase(4, unit_regroup, _latent_at(31), _regroup_at, kv)
    phase(16, unit_context, _regroup_at(3), _context_at, kv)
    phase(128, unit_window, _context_at(15),
          lambda n: jnp.minimum(_window_early(n), _window_late(n)), kv, wo)
    phase(7, unit_output, _window_late(127), _output_at, wo, issue(LAST, END, issue_last))

    @pl.loop(0, 4)
    def _(i):
        wait(wob.at[:, i, _block(7, 128)], sem_o.at[7 + i])
        for m in range(2):
            y = y_s[m] + project(m, i, 7)
            y_s[m] = y
            out_ref[:, _block(m, DM)] = y[:B].astype(BF16)


@jax.jit
def pallas_concat_heads__sliding_block_cached__compressed_kv_cla__decode_kernel(
    A_x, A_k_cache, A_v_cache, A_wq, A_wo, B_x, B_c_kv, B_w_q, B_w_uk, B_w_uv, B_w_o,
):
    vmem, dma = pltpu.VMEM, pltpu.SemaphoreType.DMA
    per_head = H * 8 + 8
    out = pl.pallas_call(
        _kernel,
        out_shape=jax.ShapeDtypeStruct((B, 2 * DM), BF16),
        in_specs=[pl.BlockSpec(memory_space=pltpu.HBM)] * 11,
        out_specs=pl.BlockSpec(memory_space=pltpu.VMEM),
        scratch_shapes=[
            vmem((32, 4, WIN, DH), BF16), vmem((32, 4, WIN, DH), BF16), vmem((2, 2, 4, SK // 4, DC), BF16),
            vmem((4, DM // 4, H * DH), BF16), vmem((2, 4, 8 * DH, DM), BF16),
            vmem((4, 128 * H, DH), BF16), vmem((4, 128 * H, DH), BF16), vmem((4, 128 * H, DH), BF16),
            vmem((2, B, DM), BF16),
            vmem((257 * PITCH + 7, DH), U32), vmem((257 * PITCH + 7, DH), U32),
            vmem((per_head, DH), F32), vmem((4, per_head, 128), F32), vmem((4, per_head, 128), F32),
            vmem((2, per_head, DH), F32),
            vmem((8, WIN), F32), vmem((8, WIN), F32), vmem((8, 128), F32),
            vmem((H, 128), F32), vmem((H, 128), F32), vmem((4, H, 128), F32), vmem((2, 8, DM), F32),
            dma((2,)), dma((4,)), dma, dma((2, 16)), dma((11,)),
        ],
        compiler_params=pltpu.CompilerParams(
            vmem_limit_bytes=120 * 1024 * 1024,
            disable_bounds_checks=True,
            disable_semaphore_checks=True,
        ),
    )(
        A_x.reshape(B, DM), A_k_cache.reshape(32, 4, SK, DH), A_v_cache.reshape(32, 4, SK, DH),
        A_wq.reshape(4, DM // 4, H * DH), A_wo.reshape(4, 8 * DH, DM),
        B_x.reshape(B, DM), B_c_kv.reshape(2, 2, 4, SK // 4, DC),
        B_w_q.reshape(4, 128 * H, DH), B_w_uk.reshape(4, 128 * H, DH), B_w_uv.reshape(4, 128 * H, DH),
        B_w_o.reshape(4, 8 * DH, DM),
    )
    return out.reshape(B, 1, 2 * DM)
```

```python
import jax
import jax.numpy as jnp
from jax import lax
import jax.experimental.pallas as pl
import jax.experimental.pallas.tpu as pltpu

B, H, DH, DM, SK, DC = 4, 32, 128, 512, 4096, 512
WIN = min(4096, max(256, SK // 4))
SCALE = DH ** -0.5
BF16, F32, U32 = jnp.bfloat16, jnp.float32, jnp.uint32

QUEUES = (0, 0, 1, 1, 0, 0, 1, 1)
W1, CKV, W2, KV, WO, LAST, END = 0, 64, 192, 256, 768, 824, 832
PITCH = H + 1


def _dot(a, b):
    return jnp.dot(a, b, preferred_element_type=F32)


def _dot_nt(a, b):
    return lax.dot_general(a, b, (((1,), (1,)), ((), ())), preferred_element_type=F32)


def _block(i, n):
    return pl.ds(i * n if isinstance(i, int) else pl.multiple_of(i * n, n), n)


def _lanes(x, n):
    return x[:, n * 128:(n + 1) * 128]


def _ramp(start, rate):
    return lambda n: start + ((n * int(rate * 64)) >> 6)


_query_at = _ramp(CKV + 16, 4.9)
_latent_at = _ramp(W2 + 16, 5)
_regroup_at = _ramp(_latent_at(31) + 2, 2)
_context_at = _ramp(_regroup_at(3) + 2, 2.5)
_window_early, _window_late = _ramp(_context_at(15) + 3, 3.08), _ramp(781 - 240, 2)
_output_at = _ramp(_window_late(127) + 6, 6)
assert _query_at(23) >= W2 and _regroup_at(0) >= KV + 8 and _context_at(15) <= WO
assert all(min(_window_early(8 * g), _window_late(8 * g)) >= KV + 32 * (g + 1) + 8 for g in range(16))
assert _window_late(127) <= min(_window_early(127), LAST)
assert all(_output_at(n) >= WO + 8 * (n + 1) + 8 for n in range(7)) and _output_at(6) >= END


def _kernel(ax_h, k_h, v_h, wq_h, wo_h, bx_h, c_h, bwq_h, wuk_h, wuv_h, bwo_h, out_ref,
            kb, vb, cb, wqb, wob, bwqb, wukb, wuvb, xb, heads0, heads1,
            qa_s, qc_s, cc_s, o_s, s_s, p_s, l_s, m_s, lc_s, acc_s, y_s,
            sem_x, sem_w, sem_c, sem_kv, sem_o):

    def burst(copy):
        count = [0, 0]
        for q in QUEUES:
            pltpu.make_async_copy(*copy(q, count[q])).start(priority=q)
            count[q] += 1

    def issue_w1(u):
        r = _block(u, 64)
        burst(lambda q, i: ((bwq_h, wuk_h)[q].at[i, r], (bwqb, wukb)[q].at[i, r], sem_w.at[q]))

    def issue_ckv(u):
        b, r = u & 1, _block(u >> 1, 16)
        burst(lambda q, i: (c_h.at[q, b, i, r], cb.at[q, b, i, r], sem_c))

    def issue_w2(u):
        r, rq, cq = _block(u, 64), _block(u >> 2, 8), _block(u & 3, 1024)
        burst(lambda q, i: (wuv_h.at[i, r], wuvb.at[i, r], sem_w.at[3]) if q else
              (wq_h.at[i, rq, cq], wqb.at[i, rq, cq], sem_w.at[2]))

    def issue_kv(u):
        h, x = u >> 5, (u >> 1) & 15
        src, dst = _block(x + (SK - WIN) // 64, 64), _block(x, 64)
        burst(lambda q, i: ((k_h, v_h)[q].at[i >> 1, u & 1, i & 1, h, src],
                            (kb, vb)[q].at[h, i & 1, i >> 1, u & 1, dst], sem_kv.at[q, h]))

    def issue_wo(u):
        r = _block(u, 16)
        burst(lambda q, i: ((wo_h, bwo_h)[q].at[i, r], wob.at[q, i, r], sem_o.at[u >> 3]))

    def issue_last(u):
        i, x = u >> 1, 56 + 4 * (u & 1)
        burst(lambda q, j: ((wo_h, bwo_h)[q].at[i, _block(x + j, 16)], wob.at[q, i, _block(x + j, 16)],
                            sem_o.at[7 + i]))

    def issue(first, last, fn):
        def run(done, target):
            pl.loop(jnp.maximum(done - first, 0), jnp.minimum(target, last) - first)(fn)
        return run

    def phase(count, unit, done, target, *streams):
        def body(n, done):
            for stream in streams:
                stream(done, target(n))
            unit(n)
            return target(n)
        lax.fori_loop(0, count, body, done)

    def wait(ref, sem):
        pltpu.make_async_copy(ref, ref, sem).wait()

    x_copies = [pltpu.make_async_copy(x, xb.at[n], sem_x.at[n]) for n, x in enumerate((ax_h, bx_h))]

    def x_rows(n):
        return jnp.concatenate([xb[n].astype(F32), jnp.zeros((8 - B, DM), F32)], axis=0).astype(BF16)

    def regroup(src, dst, i):
        for j in range(32):
            w = pltpu.bitcast(src[i >> 1, _block((i & 1) * 32 + j, 64), :], U32)
            row0, row1 = w[:16], w[16:]
            even = (row0 & jnp.uint32(0xFFFF)) | (row1 << 16)
            odd = (row0 >> 16) | (row1 & jnp.uint32(0xFFFF0000))
            dst[pl.ds((i * 32 + j) * PITCH, H), :] = jnp.concatenate([even, odd], axis=0)

    def head(w_ref, pair, j):
        return pltpu.bitcast(w_ref[pl.ds(pair + 16 * j, 256, stride=PITCH), :], BF16)

    def unit_query(n):
        @pl.when(n == 0)
        def _():
            for copy in x_copies:
                copy.wait()
            wait(bwqb, sem_w.at[0])
            wait(wukb, sem_w.at[1])

        @pl.when(n < 8)
        def _():
            regroup(bwqb, heads0, n)
            regroup(wukb, heads1, n)

        @pl.when(n >= 8)
        def _():
            x = x_rows(1)
            for j in range(2):
                q = _dot(x, head(heads0, n - 8, j)).astype(BF16)
                qc = _dot_nt(q, head(heads1, n - 8, j))
                r = _block(2 * (n - 8) + j, 8)
                for k in range(4):
                    qc_s[k, r, :] = _lanes(qc, k)
                    cc_s[k, r, :] = jnp.zeros((8, 128), F32)

    def unit_latent(n):
        b, j = n >> 3, n & 7
        heads = pl.ds(b, H, stride=8)
        pl.when(n == 0)(lambda: wait(cb, sem_c))

        @pl.when(j == 0)
        def _():
            m_s[...] = jnp.full(m_s.shape, -jnp.inf, F32)
            lc_s[...] = jnp.zeros(lc_s.shape, F32)
            acc_s[...] = jnp.zeros(acc_s.shape, F32)
        q = jnp.concatenate([qc_s[k, heads, :] for k in range(4)], axis=1).astype(BF16)
        c = cb[b >> 1, b & 1, j >> 1, _block(j & 1, 512), :]
        s = _dot_nt(q, c) * SCALE
        m_old = m_s[...]
        m_new = jnp.maximum(m_old, jnp.max(s, axis=1, keepdims=True))
        alpha = jnp.exp(m_old - m_new)
        p = [jnp.exp(_lanes(s, k) - m_new) for k in range(4)]
        m_s[...] = m_new
        lc_s[...] = alpha * lc_s[...] + ((p[0] + p[1]) + (p[2] + p[3]))
        pc = _dot(jnp.concatenate(p, axis=1).astype(BF16), c)
        for k in range(4):
            acc_s[k] = alpha * acc_s[k] + _lanes(pc, k)

        @pl.when(j == 7)
        def _():
            l = jnp.sum(lc_s[...], axis=1, keepdims=True)
            for k in range(4):
                cc_s[k, heads, :] = acc_s[k] / l

    def unit_regroup(n):
        @pl.when(n == 0)
        def _():
            wait(wqb, sem_w.at[2])
            wait(wuvb, sem_w.at[3])
        regroup(wuvb, heads0, 2 * n)
        regroup(wuvb, heads0, 2 * n + 1)

    def unit_context(n):
        q = _dot(x_rows(0), wqb[:, :, _block(n, 256)].reshape(DM, 256))
        for j in range(2):
            h = 2 * n + j
            cc = jnp.concatenate([cc_s[k, _block(h, 8), :] for k in range(4)], axis=1).astype(BF16)
            o_s[1, _block(h, 8), :] = _dot(cc, head(heads0, n, j))
            qa_s[_block(2 * (h & 15) + (h >> 4), B), :] = _lanes(q, j)[:B]

    def unit_window(n):
        h, u = n >> 3, n & 7
        hi, lo = (u >> 1) & 1, u & 1

        @pl.when(u == 0)
        def _():
            wait(kb.at[h], sem_kv.at[0, h])
            wait(vb.at[h], sem_kv.at[1, h])

        @pl.when(u < 4)
        def _():
            q = qa_s[_block(h, 8), :].astype(BF16)
            row = lax.broadcasted_iota(jnp.int32, (8, WIN), 0)
            s = s_s[...]
            for j in range(2):
                s = jnp.where(row == 2 * u + j, _dot_nt(q, kb[h, hi, lo, j]), s)
            s_s[...] = s

        @pl.when(u == 3)
        def _():
            s = s_s[...] * SCALE
            p = jnp.exp(s - jnp.max(s, axis=1, keepdims=True))
            l_s[...] = jnp.broadcast_to(jnp.sum(p, axis=1, keepdims=True), l_s.shape)
            p_s[...] = p
            o_s[0, _block(h, 8), :] = jnp.zeros((8, DH), F32)
            o_s[0, _block(h + 16, 8), :] = jnp.zeros((8, DH), F32)

        @pl.when(u >= 4)
        def _():
            p = p_s[...].astype(BF16)
            row = lax.broadcasted_iota(jnp.int32, (8, DH), 0)
            own = _block(2 * (h + 16 * hi), B)
            o = jnp.concatenate([o_s[0, own, :]] * 2, axis=0)
            for j in range(2):
                o = jnp.where(row == 2 * (u - 4) + j, _dot(p, vb[h, hi, lo, j]) / l_s[...], o)
            o_s[0, own, :] = jnp.where(hi == 0, o[:B], o[B:])

    def project(m, i, n):
        return _dot(o_s[m, _block(8 * i + n, 8), :].astype(BF16), wob[m, i, _block(n, 128), :])

    def unit_output(n):
        wait(wob.at[:, :, _block(n, 128)], sem_o.at[n])
        for m in range(2):
            y_s[m] += (project(m, 0, n) + project(m, 1, n)) + (project(m, 2, n) + project(m, 3, n))

    @pl.loop(W1, CKV)
    def _(u):
        issue_w1(u)

        @pl.when(u == 7)
        def _():
            for n, copy in enumerate(x_copies):
                copy.start(priority=n)

    y_s[...] = jnp.zeros(y_s.shape, F32)
    s_s[...] = jnp.zeros(s_s.shape, F32)
    kv, wo = issue(KV, WO, issue_kv), issue(WO, LAST, issue_wo)
    phase(24, unit_query, CKV, _query_at, issue(CKV, W2, issue_ckv))
    phase(32, unit_latent, W2, _latent_at, issue(W2, KV, issue_w2), kv)
    phase(4, unit_regroup, _latent_at(31), _regroup_at, kv)
    phase(16, unit_context, _regroup_at(3), _context_at, kv)
    phase(128, unit_window, _context_at(15),
          lambda n: jnp.minimum(_window_early(n), _window_late(n)), kv, wo)
    phase(7, unit_output, _window_late(127), _output_at, wo, issue(LAST, END, issue_last))

    @pl.loop(0, 4)
    def _(i):
        wait(wob.at[:, i, _block(7, 128)], sem_o.at[7 + i])
        for m in range(2):
            y = y_s[m] + project(m, i, 7)
            y_s[m] = y
            out_ref[:, _block(m, DM)] = y[:B].astype(BF16)


@jax.jit
def pallas_concat_heads__sliding_block_cached__compressed_kv_cla__decode_kernel(
    A_x, A_k_cache, A_v_cache, A_wq, A_wo, B_x, B_c_kv, B_w_q, B_w_uk, B_w_uv, B_w_o,
):
    vmem, dma = pltpu.VMEM, pltpu.SemaphoreType.DMA
    per_head = H * 8 + 8
    out = pl.pallas_call(
        _kernel,
        out_shape=jax.ShapeDtypeStruct((B, 2 * DM), BF16),
        in_specs=[pl.BlockSpec(memory_space=pltpu.HBM)] * 11,
        out_specs=pl.BlockSpec(memory_space=pltpu.VMEM),
        scratch_shapes=[
            vmem((16, 2, 2, 2, WIN, DH), BF16), vmem((16, 2, 2, 2, WIN, DH), BF16),
            vmem((2, 2, 4, SK // 4, DC), BF16),
            vmem((4, DM // 4, H * DH), BF16), vmem((2, 4, 8 * DH, DM), BF16),
            vmem((4, 128 * H, DH), BF16), vmem((4, 128 * H, DH), BF16), vmem((4, 128 * H, DH), BF16),
            vmem((2, B, DM), BF16),
            vmem((257 * PITCH + 7, DH), U32), vmem((257 * PITCH + 7, DH), U32),
            vmem((H * B, DH), F32), vmem((4, per_head, 128), F32), vmem((4, per_head, 128), F32),
            vmem((2, H * 8, DH), F32),
            vmem((8, WIN), F32), vmem((8, WIN), F32), vmem((8, 128), F32),
            vmem((H, 128), F32), vmem((H, 128), F32), vmem((4, H, 128), F32), vmem((2, 8, DM), F32),
            dma((2,)), dma((4,)), dma, dma((2, 16)), dma((11,)),
        ],
        compiler_params=pltpu.CompilerParams(
            vmem_limit_bytes=120 * 1024 * 1024,
            disable_bounds_checks=True,
            disable_semaphore_checks=True,
        ),
    )(
        A_x.reshape(B, DM), A_k_cache.reshape(2, 2, 2, 16, SK, DH), A_v_cache.reshape(2, 2, 2, 16, SK, DH),
        A_wq.reshape(4, DM // 4, H * DH), A_wo.reshape(4, 8 * DH, DM),
        B_x.reshape(B, DM), B_c_kv.reshape(2, 2, 4, SK // 4, DC),
        B_w_q.reshape(4, 128 * H, DH), B_w_uk.reshape(4, 128 * H, DH), B_w_uv.reshape(4, 128 * H, DH),
        B_w_o.reshape(4, 8 * DH, DM),
    )
    return out.reshape(B, 1, 2 * DM)
```
